```python
import os as _os
_os.environ.setdefault('JAX_PLATFORMS', 'cpu')
import jax
import jax.numpy as jnp

def _softmax(x, axis=-1):
    return jax.nn.softmax(x, axis=axis)

def _gelu(x):
    return jax.nn.gelu(x, approximate=True)

def _silu(x):
    return jax.nn.silu(x)

def _sigmoid(x):
    return jax.nn.sigmoid(x)

def _layernorm(x, axis=-1, eps=1e-05):
    m = jnp.mean(x, axis=axis, keepdims=True)
    v = jnp.var(x, axis=axis, keepdims=True)
    return (x - m) / jnp.sqrt(v + eps)

def _scatter_add(tgt, idx, src, axis=0):
    return tgt.at[idx].add(src)

def _segment_sum(src, seg, n):
    return jax.ops.segment_sum(src, seg, n)

class _Rng:

    def __init__(self, key):
        self._k = key

    def _next(self):
        self._k, sub = jax.random.split(self._k)
        return sub

    def normal(self, shape):
        return jax.random.normal(self._next(), shape, dtype=jnp.bfloat16)

    def randint(self, lo, hi, shape):
        return jax.random.randint(self._next(), shape, lo, hi, dtype=jnp.int32)

    def uniform(self, shape, lo=0.0, hi=1.0):
        return jax.random.uniform(self._next(), shape, jnp.bfloat16, lo, hi)

    def permutation(self, n):
        return jax.random.permutation(self._next(), n)
kernel_name = 'adaLN_cond__mha_block__geglu_ffn__prompt'

def setup_inputs():
    _rng = _Rng(jax.random.key(int.from_bytes(__import__("os").urandom(4), "little")))
    _w = lambda a: (lambda t: t.astype(jnp.bfloat16) if jnp.issubdtype(t.dtype, jnp.floating) else t)(jnp.asarray(a))

    def _A_setup():
        B, S, D, H = (1, 2048, 640, 32)
        return {'x': _w((lambda *s: _rng.normal(s) * 0.05)(B, S, D)), 'wqkv': _w((lambda *s: _rng.normal(s) * 0.05)(D, 3 * D)), 'wo': _w((lambda *s: _rng.normal(s) * 0.05)(D, D))}
    _A_in = _A_setup()

    def _B_setup():
        B, S, D, F = (1, 2048, 640, 1728)
        return {'x': _w((lambda *s: _rng.normal(s) * 0.05)(B, S, D)), 'w_gate': _w((lambda *s: _rng.normal(s) * 0.05)(D, F)), 'w_up': _w((lambda *s: _rng.normal(s) * 0.05)(D, F)), 'w_down': _w((lambda *s: _rng.normal(s) * 0.05)(F, D))}
    _B_in = _B_setup()
    return {'A_x': _A_in['x'], 'A_wqkv': _A_in['wqkv'], 'A_wo': _A_in['wo'], 'B_x': _B_in['x'], 'B_w_gate': _B_in['w_gate'], 'B_w_up': _B_in['w_up'], 'B_w_down': _B_in['w_down'], 'c': _w((lambda *s: _rng.normal(s) * 0.05)(1, 640) * 8.0), 'w_mod': _w((lambda *s: _rng.normal(s) * 0.05)(640, 6 * 640) * 640 ** (-0.5) * 8.0)}

def reference(A_x, A_wqkv, A_wo, B_x, B_w_gate, B_w_up, B_w_down, c, w_mod):

    def _A_ref(x, wqkv, wo):
        B, S, D = x.shape
        H = 32
        Dh = D // H
        qkv = (lambda x, *d: x.transpose(*d))((x @ wqkv).reshape(B, S, 3, H, Dh), 2, 0, 3, 1, 4)
        q, k, v = (qkv[0], qkv[1], qkv[2])
        scores = jnp.einsum('bhqd,bhkd->bhqk', q, k) * Dh ** (-0.5)
        p = _softmax(scores, axis=-1)
        o = jnp.einsum('bhqk,bhkd->bhqd', p, v)
        return (lambda x, *d: x.transpose(*d))(o, 0, 2, 1, 3).reshape(B, S, D) @ wo

    def _B_ref(x, w_gate, w_up, w_down):
        return _gelu(x @ w_gate) * (x @ w_up) @ w_down
    x = A_x
    mod = (_silu(c) @ w_mod).reshape(c.shape[0], 6, 1, -1)
    sa, ca, ga, sb, cb, gb = (mod[:, 0].copy(), mod[:, 1].copy(), mod[:, 2].copy(), mod[:, 3].copy(), mod[:, 4].copy(), mod[:, 5].copy())
    h = _layernorm(x, axis=-1) * (1 + ca) + sa
    x = x + ga * _A_ref(h, A_wqkv, A_wo)
    h = _layernorm(x, axis=-1) * (1 + cb) + sb
    x = x + gb * _B_ref(h, B_w_gate, B_w_up, B_w_down)
    return x
```

```python
import jax
import jax.numpy as jnp
from jax import lax
import jax.experimental.pallas as pl
import jax.experimental.pallas.tpu as pltpu

S = 2048
D = 640
H = 32
DH = 20
F = 1728
EPS = 1e-5
LANES = 128
NG = 6
HP = 24
VP = 32
TQ = 512
CK = 128
NQB = S // TQ
NC = S // CK
NSTEP = H * NQB
TM1 = 256
TM3 = 128
STRADDLE = (6, 12, 19, 25)
QSCALE = float(DH) ** -0.5 * 1.4426950408889634

F32 = jnp.float32
BF16 = jnp.bfloat16
NT = (((1,), (1,)), ((), ()))
TN = (((0,), (0,)), ((), ()))


def _layernorm(x):
    mu = jnp.mean(x, axis=-1, keepdims=True)
    xc = x - mu
    var = jnp.mean(xc * xc, axis=-1, keepdims=True)
    return xc * lax.rsqrt(var + EPS)


def _gelu(x):
    c = 0.7978845608028654
    return 0.5 * x * (1.0 + jnp.tanh(c * (x + 0.044715 * (x * x * x))))


def _kernel(x_hbm, wqkv_hbm, wo_hbm, wg_hbm, wu_hbm, wd_hbm, c_hbm, wmod_hbm,
            out_hbm,
            x_v, wqkv_v, wo_v, wg_v, wu_v, wd_v, c_v, wmod_v, out_v,
            mod_v, wkx_v, wqvt_v, wop_v,
            k_s, qt_s, vt_s, s0, s1, m0, m1, q0, q1, at_s,
            in_sems, out_sems):
    def cp(src, dst, i):
        return pltpu.make_async_copy(src, dst, in_sems.at[i])

    c_cp = cp(c_hbm, c_v, 0)
    wmod_a = cp(wmod_hbm.at[:, 0:2 * D], wmod_v.at[:, 0:2 * D], 1)
    x_cp = cp(x_hbm, x_v, 2)
    wqkv_cp = cp(wqkv_hbm, wqkv_v, 3)
    wmod_b = cp(wmod_hbm.at[:, 2 * D:6 * D], wmod_v.at[:, 2 * D:6 * D], 4)
    wo_cp = cp(wo_hbm, wo_v, 5)
    wg_cp = cp(wg_hbm, wg_v, 6)
    wu_cp = cp(wu_hbm, wu_v, 7)
    wd_cp = cp(wd_hbm, wd_v, 8)
    c_cp.start()
    wmod_a.start()
    wqkv_cp.start()
    x_cp.start()

    wqkv_cp.wait()
    wq = wqkv_v[:, 0:D].astype(F32)
    wk = wqkv_v[:, D:2 * D].astype(F32)
    zpad = jnp.zeros((D, LANES - DH * len(STRADDLE)), F32)
    wkx_v[...] = jnp.concatenate(
        [wk[:, h * DH:(h + 1) * DH] for h in STRADDLE] + [zpad], axis=1).astype(BF16)
    wqx = jnp.concatenate(
        [wq[:, h * DH:(h + 1) * DH] for h in STRADDLE] + [zpad], axis=1)
    wqvt_v[0:D, :] = wq.T.astype(BF16)
    wqvt_v[D:D + LANES, :] = wqx.T.astype(BF16)
    wqvt_v[D + LANES:, :] = wqkv_v[:, 2 * D:3 * D].astype(F32).T.astype(BF16)

    wmod_b.start()
    wo_cp.start()
    wg_cp.start()
    wu_cp.start()
    wd_cp.start()

    c_cp.wait()
    cf = c_v[...].astype(F32)
    sc = (cf * jax.nn.sigmoid(cf)).astype(BF16)
    sc16 = jnp.broadcast_to(sc, (16, D))
    wmod_a.wait()
    mod_v[:, 0:2 * D] = jnp.dot(sc16, wmod_v[:, 0:2 * D], preferred_element_type=F32)

    x_cp.wait()

    def phase1(r, carry):
        r0 = pl.multiple_of(r * TM1, TM1)
        rows = pl.ds(r0, TM1)
        sa = mod_v[0:1, 0:D]
        ca = mod_v[0:1, D:2 * D]
        hb = (_layernorm(x_v[rows, :].astype(F32)) * (1.0 + ca) + sa).astype(BF16)
        kk = jnp.dot(hb, wqkv_v[:, D:2 * D], preferred_element_type=F32)
        for g in range(NG - 1):
            k_s[g, rows, :] = kk[:, g * LANES:(g + 1) * LANES].astype(BF16)
        k_s[NG - 1, rows, :] = jnp.dot(hb, wkx_v[...], preferred_element_type=F32).astype(BF16)
        qv = lax.dot_general(wqvt_v[...], hb, NT, preferred_element_type=F32)
        qt_s[:, rows] = (qv[0:NG * LANES, :] * QSCALE).astype(BF16)
        tail = jnp.where(lax.broadcasted_iota(jnp.int32, (VP - DH, TM1), 0) == 0, 1.0, 0.0).astype(F32)
        for h in range(H):
            v0 = NG * LANES + h * DH
            vt_s[h, :, rows] = jnp.concatenate([qv[v0:v0 + DH, :], tail], axis=0).astype(BF16)
        return carry

    lax.fori_loop(0, S // TM1, phase1, 0)

    wmod_b.wait()
    mod_v[:, 2 * D:6 * D] = jnp.dot(sc16, wmod_v[:, 2 * D:6 * D], preferred_element_type=F32)
    wo_cp.wait()
    wo = wo_v[...].astype(F32)
    zrow = jnp.zeros((HP - DH, D), F32)
    for h in range(H):
        wop_v[h * HP:(h + 1) * HP, :] = jnp.concatenate(
            [wo[h * DH:(h + 1) * DH, :], zrow], axis=0).astype(BF16)
    wg_cp.wait()
    wu_cp.wait()
    wd_cp.wait()

    s_refs = (s0, s1)
    m_refs = (m0, m1)
    q_refs = (q0, q1)

    def head_loc(h):
        c0 = h * DH
        g = c0 // LANES
        straddle = (c0 + DH - 1) // LANES != g
        return jnp.where(straddle, NG - 1, g), jnp.where(straddle, g * DH, c0 - g * LANES)

    def prep_q(i, q_ref):
        i = jnp.minimum(i, NSTEP - 1)
        h = i % H
        qb = i // H
        g, off = head_loc(h)
        g0 = pl.multiple_of(g * LANES, LANES)
        qt = qt_s[pl.ds(g0, LANES), pl.ds(pl.multiple_of(qb * TQ, TQ), TQ)]
        row = lax.broadcasted_iota(jnp.int32, (LANES, TQ), 0)
        q_ref[...] = jnp.where((row >= off) & (row < off + DH), qt, jnp.zeros_like(qt))

    def step(ia, sa_ref, ma_ref, qa_ref, ib, sb_ref, mb_ref):
        if ia is not None:
            g, _ = head_loc(ia % H)
            macc = None
        if ib is not None:
            hb = ib % H
            mb = mb_ref[...]
            oacc = None
        for c in range(NC):
            if ia is not None:
                s = jnp.dot(k_s[g, c * CK:(c + 1) * CK, :], qa_ref[...], preferred_element_type=F32)
                sa_ref[c * CK:(c + 1) * CK, :] = s
                mm = jnp.max(s.reshape(CK // 8, 8, TQ), axis=0)
                macc = mm if macc is None else jnp.maximum(macc, mm)
            if ib is not None:
                p = jnp.exp2(sb_ref[c * CK:(c + 1) * CK, :] - mb).astype(BF16)
                o = jnp.dot(vt_s[hb, :, c * CK:(c + 1) * CK], p, preferred_element_type=F32)
                oacc = o if oacc is None else oacc + o
        if ia is not None:
            ma_ref[...] = jnp.max(macc, axis=0, keepdims=True)
        if ib is not None:
            at_s[hb] = oacc[0:HP, :] * (1.0 / oacc[DH:DH + 1, :])

    def out_cp(blk):
        r0 = pl.multiple_of(blk * TM3, TM3)
        return pltpu.make_async_copy(out_v.at[pl.ds(r0, TM3), :], out_hbm.at[pl.ds(r0, TM3), :],
                                     out_sems.at[blk])

    def phase3(qb):
        def sub(j, carry):
            blk = qb * (TQ // TM3) + j
            rows = pl.ds(pl.multiple_of(blk * TM3, TM3), TM3)
            ga = mod_v[0:1, 2 * D:3 * D]
            sb = mod_v[0:1, 3 * D:4 * D]
            cb = mod_v[0:1, 4 * D:5 * D]
            gb = mod_v[0:1, 5 * D:6 * D]
            a_t = at_s[:, :, pl.ds(pl.multiple_of(j * TM3, TM3), TM3)].reshape(H * HP, TM3).astype(BF16)
            y = lax.dot_general(a_t, wop_v[...], TN, preferred_element_type=F32)
            x1 = x_v[rows, :].astype(F32) + ga * y
            h2 = (_layernorm(x1) * (1.0 + cb) + sb).astype(BF16)
            gate = lax.dot_general(h2, wg_v[...], NT, preferred_element_type=F32)
            up = lax.dot_general(h2, wu_v[...], NT, preferred_element_type=F32)
            act = (_gelu(gate) * up).astype(BF16)
            y2 = jnp.dot(act, wd_v[...], preferred_element_type=F32)
            out_v[rows, :] = (x1 + gb * y2).astype(BF16)
            out_cp(blk).start()
            return carry
        lax.fori_loop(0, TQ // TM3, sub, 0)

    prep_q(0, q0)
    prep_q(1, q1)
    step(0, s0, m0, q0, None, None, None)

    def body(j, carry):
        i = 2 * j
        for u in range(2):
            a, b = (u + 1) % 2, u % 2
            prep_q(i + u + 2, q_refs[b])
            step(i + u + 1, s_refs[a], m_refs[a], q_refs[a], i + u, s_refs[b], m_refs[b])

        @pl.when((i + 1) % H == H - 1)
        def _():
            phase3((i + 1) // H)
        return carry

    lax.fori_loop(0, NSTEP // 2 - 1, body, 0)
    i = NSTEP - 2
    step(i + 1, s1, m1, q1, i, s0, m0)
    step(None, None, None, None, i + 1, s1, m1)
    phase3(NQB - 1)

    for blk in range(S // TM3):
        out_cp(blk).wait()


@jax.jit
def pallas_adaLN_cond__mha_block__geglu_ffn__prompt_kernel(
    A_x: jax.Array,
    A_wqkv: jax.Array,
    A_wo: jax.Array,
    B_x: jax.Array,
    B_w_gate: jax.Array,
    B_w_up: jax.Array,
    B_w_down: jax.Array,
    c: jax.Array,
    w_mod: jax.Array,
):
    del B_x
    x = A_x.reshape(S, D)
    any_spec = pl.BlockSpec(memory_space=pltpu.HBM)
    vm = pltpu.VMEM
    out = pl.pallas_call(
        _kernel,
        out_shape=jax.ShapeDtypeStruct((S, D), BF16),
        in_specs=[any_spec] * 8,
        out_specs=any_spec,
        scratch_shapes=[
            vm((S, D), BF16),
            vm((D, 3 * D), BF16),
            vm((D, D), BF16),
            vm((F, D), BF16),
            vm((F, D), BF16),
            vm((F, D), BF16),
            vm((1, D), BF16),
            vm((D, 6 * D), BF16),
            vm((S, D), BF16),
            vm((16, 6 * D), F32),
            vm((D, LANES), BF16),
            vm((NG * LANES + D, D), BF16),
            vm((H * HP, D), BF16),
            vm((NG, S, LANES), BF16),
            vm((NG * LANES, S), BF16),
            vm((H, VP, S), BF16),
            vm((S, TQ), F32),
            vm((S, TQ), F32),
            vm((1, TQ), F32),
            vm((1, TQ), F32),
            vm((LANES, TQ), BF16),
            vm((LANES, TQ), BF16),
            vm((H, HP, TQ), F32),
            pltpu.SemaphoreType.DMA((9,)),
            pltpu.SemaphoreType.DMA((S // TM3,)),
        ],
        compiler_params=pltpu.CompilerParams(vmem_limit_bytes=100 * 1024 * 1024),
    )(x, A_wqkv, A_wo, B_w_gate.T, B_w_up.T, B_w_down, c, w_mod)
    return out.reshape(1, S, D)
```

```python
import jax
import jax.numpy as jnp
from jax import lax
import jax.experimental.pallas as pl
import jax.experimental.pallas.tpu as pltpu

S = 2048
D = 640
H = 32
DH = 20
F = 1728
FM = 1664
FT = F - FM
EPS = 1e-5
LANES = 128
NG = D // LANES
NKG = NG + 4
HP = 24
VP = 32
TQ = 512
CK = 128
NQB = S // TQ
NC = S // CK
NSTEP = H * NQB
UN = 8
DEPLAG = 3
TM1 = 256
NB1 = S // TM1
TM3 = 128
NB3 = S // TM3
STRADDLE = (6, 12, 19, 25)
QSCALE = float(DH) ** -0.5 * 1.4426950408889634

F32 = jnp.float32
BF16 = jnp.bfloat16
U32 = jnp.uint32


def _pack(x):
    return pltpu.bitcast(x, U32)


def _unpack(x):
    return pltpu.bitcast(x, BF16)


NT = (((1,), (1,)), ((), ()))
TN = (((0,), (0,)), ((), ()))


def _layernorm(x):
    mu = jnp.mean(x, axis=-1, keepdims=True)
    xc = x - mu
    var = jnp.mean(xc * xc, axis=-1, keepdims=True)
    return xc * lax.rsqrt(var + EPS)


def _gelu(x):
    c = 0.7978845608028654
    return 0.5 * x * (1.0 + jnp.tanh(c * (x + 0.044715 * (x * x * x))))


def _kernel(x_hbm, wqkv_hbm, wo_hbm, wg_hbm, wu_hbm, wd_hbm, c_hbm, wmod_hbm,
            out_hbm,
            x_v, wqkv_v, wo_v, wg_v, wu_v, wt_v, wd_v, c_v, wmod_v, out_v,
            mod_v, wqvt_v, h_all,
            h0, h1, x10, x11,
            k_s, qt_s, vt_s, s0, s1, m0, m1, q0, q1, at_s,
            in_sems, out_sems):
    def cp(src, dst, i):
        return pltpu.make_async_copy(src, dst, in_sems.at[i])

    XA = 2 * TM1

    xa_cp = cp(x_hbm.at[0:XA, :], x_v.at[0:XA, :], 12)
    xb_cp = cp(x_hbm.at[XA:S, :], x_v.at[XA:S, :], 13)
    c_cp = cp(c_hbm, c_v, 0)
    wmod_a = cp(wmod_hbm.at[:, 0:2 * D], wmod_v.at[:, 0:2 * D], 1)
    wk_cp = cp(wqkv_hbm.at[:, D:2 * D], wqkv_v.at[:, D:2 * D], 2)
    wq_cp = cp(wqkv_hbm.at[:, 0:D], wqkv_v.at[:, 0:D], 3)
    wv_cp = cp(wqkv_hbm.at[:, 2 * D:3 * D], wqkv_v.at[:, 2 * D:3 * D], 4)
    wmod_b = cp(wmod_hbm.at[:, 2 * D:6 * D], wmod_v.at[:, 2 * D:6 * D], 5)
    wo_cp = cp(wo_hbm, wo_v, 6)
    wg_cp = cp(wg_hbm, wg_v, 7)
    wu_cp = cp(wu_hbm, wu_v, 8)
    wd_cp = cp(wd_hbm, wd_v, 9)
    wtg_cp = cp(wg_hbm.at[FM:F, :], wt_v.at[0:FT, :], 10)
    wtu_cp = cp(wu_hbm.at[FM:F, :], wt_v.at[FT:2 * FT, :], 11)
    c_cp.start()
    wmod_a.start()
    xa_cp.start()
    wk_cp.start()

    c_cp.wait()
    cf = c_v[...].astype(F32)
    sc = (cf * jax.nn.sigmoid(cf)).astype(BF16)
    sc16 = jnp.broadcast_to(sc, (16, D))
    wmod_a.wait()
    xb_cp.start()
    wq_cp.start()
    wv_cp.start()
    mod_v[:, 0:2 * D] = jnp.dot(sc16, wmod_v[:, 0:2 * D], preferred_element_type=F32)

    def ln1(r):
        rows = pl.ds(r * TM1, TM1)
        sa = mod_v[0:1, 0:D]
        ca = mod_v[0:1, D:2 * D]
        h_all[rows, :] = (_layernorm(x_v[rows, :].astype(F32)) * (1.0 + ca) + sa).astype(BF16)

    def kproj(r):
        rows = pl.ds(r * TM1, TM1)
        prow = pl.ds(r * (TM1 // 2), TM1 // 2)
        kk = jnp.dot(h_all[rows, :], wqkv_v[:, D:2 * D], preferred_element_type=F32)
        kg = [kk[:, g * LANES:(g + 1) * LANES] for g in range(NG)]
        for g in range(NG):
            k_s[g, prow, :] = _pack(kg[g].astype(BF16))
        lane = lax.broadcasted_iota(jnp.int32, (TM1, LANES), 1)
        for i, h in enumerate(STRADDLE):
            g, lo = divmod(h * DH, LANES)
            k_s[NG + i, prow, :] = _pack(jnp.where(lane >= lo, kg[g], kg[g + 1]).astype(BF16))

    xa_cp.wait()
    wk_cp.wait()
    ln1(0)
    ln1(1)
    kproj(0)
    kproj(1)
    xb_cp.wait()
    wq_cp.wait()
    wv_cp.wait()
    wmod_b.start()
    wo_cp.start()
    wg_cp.start()
    wu_cp.start()
    wd_cp.start()
    wtg_cp.start()
    wtu_cp.start()
    for r in range(2, NB1):
        ln1(r)
        kproj(r)
        if r == 3:
            wqvt_v[0:D, :] = wqkv_v[:, 0:D].T
            wqvt_v[D:2 * D, :] = wqkv_v[:, 2 * D:3 * D].T

    def qvproj(r, carry):
        rows = pl.ds(pl.multiple_of(r * TM1, TM1), TM1)
        qv = lax.dot_general(wqvt_v[...], h_all[rows, :], NT, preferred_element_type=F32)
        q = qv[0:D, :] * QSCALE
        qt_s[:, rows] = q.astype(BF16)
        tail = jnp.where(lax.broadcasted_iota(jnp.int32, (VP - DH, TM1), 0) == 0, 1.0, 0.0).astype(F32)
        for h in range(H):
            v0 = D + h * DH
            vt_s[h, :, rows] = _pack(jnp.concatenate([qv[v0:v0 + DH, :], tail], axis=0).astype(BF16))
        return carry

    lax.fori_loop(0, NB1, qvproj, 0)

    wmod_b.wait()
    wo_cp.wait()
    wg_cp.wait()
    wu_cp.wait()
    wd_cp.wait()
    wtg_cp.wait()
    wtu_cp.wait()
    mod_v[:, 2 * D:6 * D] = jnp.dot(sc16, wmod_v[:, 2 * D:6 * D], preferred_element_type=F32)

    s_refs = (s0, s1)
    m_refs = (m0, m1)
    q_refs = (q0, q1)

    def k_group(h):
        g = (h * DH) // LANES
        straddle = (h * DH + DH - 1) // LANES != g
        return jnp.where(straddle, NG + g, g)

    def prep_q(i, q_ref):
        i = jnp.minimum(i, NSTEP - 1)
        h = i // NQB
        qb = i % NQB
        c0 = h * DH
        g = c0 // LANES
        g2 = (c0 + DH - 1) // LANES
        lo = c0 - g * LANES
        cols = pl.ds(pl.multiple_of(qb * TQ, TQ), TQ)
        qa = qt_s[pl.ds(pl.multiple_of(g * LANES, LANES), LANES), cols]
        qb_ = qt_s[pl.ds(pl.multiple_of(g2 * LANES, LANES), LANES), cols]
        row = lax.broadcasted_iota(jnp.int32, (LANES, TQ), 0)
        zero = jnp.zeros_like(qa)
        q_ref[...] = _pack(jnp.where((row >= lo) & (row < lo + DH), qa,
                                     jnp.where(row < lo + DH - LANES, qb_, zero)))

    def step(ia, sa_ref, ma_ref, qa_ref, ib, sb_ref, mb_ref):
        if ia is not None:
            g = k_group(ia // NQB)
            macc = None
            mhist = []
        if ib is not None:
            hb = ib // NQB
            qb = ib % NQB
            mb = jnp.broadcast_to(mb_ref[...], (8, TQ))
            oacc = None
        for c in range(NC):
            if ia is not None:
                kc = _unpack(k_s[g, c * (CK // 2):(c + 1) * (CK // 2), :])
                s = jnp.dot(kc, _unpack(qa_ref[...]), preferred_element_type=F32)
                sa_ref[c * CK:(c + 1) * CK, :] = s
                mm = jnp.max(s.reshape(CK // 8, 8, TQ), axis=0)
                macc = mm if macc is None else jnp.maximum(macc, mm)
                mhist.append(macc)
            if ib is None:
                continue
            mbb = mb
            if ia is not None and c >= DEPLAG:
                mbb = jnp.maximum(mb, jnp.minimum(mhist[c - DEPLAG], mb))
            sc_ = sb_ref[c * CK:(c + 1) * CK, :].reshape(CK // 8, 8, TQ)
            p = jnp.exp2(sc_ - mbb[None]).reshape(CK, TQ).astype(BF16)
            o = jnp.dot(_unpack(vt_s[hb, :, c * CK:(c + 1) * CK]), p, preferred_element_type=F32)
            oacc = o if oacc is None else oacc + o
        if ia is not None:
            ma_ref[...] = jnp.max(macc, axis=0, keepdims=True)
        if ib is not None:
            at_s[hb, :, pl.ds(pl.multiple_of(qb * TQ, TQ), TQ)] = oacc[0:HP, :] * (1.0 / oacc[DH:DH + 1, :])

    prep_q(0, q0)
    prep_q(1, q1)
    step(0, s0, m0, q0, None, None, None)

    def body(j, carry):
        i = UN * j
        for u in range(UN):
            a, b = (u + 1) % 2, u % 2
            prep_q(i + u + 2, q_refs[b])
            step(i + u + 1, s_refs[a], m_refs[a], q_refs[a], i + u, s_refs[b], m_refs[b])
        return carry

    lax.fori_loop(0, NSTEP // UN - 1, body, 0)
    i = NSTEP - UN
    for u in range(UN):
        a, b = (u + 1) % 2, u % 2
        if u + 1 < UN:
            if u + 2 < UN:
                prep_q(i + u + 2, q_refs[b])
            step(i + u + 1, s_refs[a], m_refs[a], q_refs[a], i + u, s_refs[b], m_refs[b])
        else:
            step(None, None, None, None, i + u, s_refs[b], m_refs[b])

    h_refs = (h0, h1)
    x1_refs = (x10, x11)

    def out_cp(blk):
        r0 = pl.multiple_of(blk * TM3, TM3)
        return pltpu.make_async_copy(out_v.at[pl.ds(r0, TM3), :], out_hbm.at[pl.ds(r0, TM3), :],
                                     out_sems.at[blk])

    def stage_x(blk, h_ref, x1_ref):
        blk = jnp.minimum(blk, NB3 - 1)
        rows = pl.ds(pl.multiple_of(blk * TM3, TM3), TM3)
        ga = mod_v[0:1, 2 * D:3 * D]
        sb = mod_v[0:1, 3 * D:4 * D]
        cb = mod_v[0:1, 4 * D:5 * D]
        a_t = jnp.concatenate([at_s[h, 0:DH, rows] for h in range(H)], axis=0).astype(BF16)
        y = lax.dot_general(a_t, wo_v[...], TN, preferred_element_type=F32)
        x1 = x_v[rows, :].astype(F32) + ga * y
        x1_ref[...] = x1
        h_ref[...] = (_layernorm(x1) * (1.0 + cb) + sb).astype(BF16)

    def stage_y(blk, h_ref, x1_ref):
        rows = pl.ds(pl.multiple_of(blk * TM3, TM3), TM3)
        gb = mod_v[0:1, 5 * D:6 * D]
        h2 = h_ref[...]
        gate = lax.dot_general(h2, wg_v[0:FM, :], NT, preferred_element_type=F32)
        up = lax.dot_general(h2, wu_v[0:FM, :], NT, preferred_element_type=F32)
        gu = lax.dot_general(h2, wt_v[...], NT, preferred_element_type=F32)
        act = (_gelu(gate) * up).astype(BF16)
        act_t = (_gelu(gu) * pltpu.roll(gu, FT, 1))[:, 0:FT].astype(BF16)
        y2 = jnp.dot(act, wd_v[0:FM, :], preferred_element_type=F32)
        y2 = y2 + jnp.dot(act_t, wd_v[FM:F, :], preferred_element_type=F32)
        out_v[rows, :] = (x1_ref[...] + gb * y2).astype(BF16)
        out_cp(blk).start()

    stage_x(0, h0, x10)

    def phase3(j, carry):
        for u in range(2):
            stage_x(2 * j + u + 1, h_refs[1 - u], x1_refs[1 - u])
            stage_y(2 * j + u, h_refs[u], x1_refs[u])
        return carry

    lax.fori_loop(0, NB3 // 2, phase3, 0)

    for blk in range(NB3):
        out_cp(blk).wait()


@jax.jit
def pallas_adaLN_cond__mha_block__geglu_ffn__prompt_kernel(
    A_x: jax.Array,
    A_wqkv: jax.Array,
    A_wo: jax.Array,
    B_x: jax.Array,
    B_w_gate: jax.Array,
    B_w_up: jax.Array,
    B_w_down: jax.Array,
    c: jax.Array,
    w_mod: jax.Array,
):
    del B_x
    x = A_x.reshape(S, D)
    hbm = pl.BlockSpec(memory_space=pltpu.HBM)
    vm = pltpu.VMEM
    out = pl.pallas_call(
        _kernel,
        out_shape=jax.ShapeDtypeStruct((S, D), BF16),
        in_specs=[hbm] * 8,
        out_specs=hbm,
        scratch_shapes=[
            vm((S, D), BF16),
            vm((D, 3 * D), BF16),
            vm((D, D), BF16),
            vm((F, D), BF16),
            vm((F, D), BF16),
            vm((2 * FT, D), BF16),
            vm((F, D), BF16),
            vm((1, D), BF16),
            vm((D, 6 * D), BF16),
            vm((S, D), BF16),
            vm((16, 6 * D), F32),
            vm((2 * D, D), BF16),
            vm((S, D), BF16),
            vm((TM3, D), BF16),
            vm((TM3, D), BF16),
            vm((TM3, D), F32),
            vm((TM3, D), F32),
            vm((NKG, S // 2, LANES), U32),
            vm((D, S), BF16),
            vm((H, VP // 2, S), U32),
            vm((S, TQ), F32),
            vm((S, TQ), F32),
            vm((1, TQ), F32),
            vm((1, TQ), F32),
            vm((LANES // 2, TQ), U32),
            vm((LANES // 2, TQ), U32),
            vm((H, HP, S), F32),
            pltpu.SemaphoreType.DMA((14,)),
            pltpu.SemaphoreType.DMA((NB3,)),
        ],
        compiler_params=pltpu.CompilerParams(vmem_limit_bytes=100 * 1024 * 1024),
    )(x, A_wqkv, A_wo, B_w_gate.T, B_w_up.T, B_w_down, c, w_mod)
    return out.reshape(1, S, D)
```

```python
import jax
import jax.numpy as jnp
from jax import lax
import jax.experimental.pallas as pl
import jax.experimental.pallas.tpu as pltpu

S = 2048
D = 640
H = 32
DH = 20
F = 1728
FM = 1664
FT = F - FM
EPS = 1e-5
FCW = 256
XPOS = 2
FCH = [(FM, F)] + [(f, min(f + FCW, FM)) for f in range(0, FM, FCW)]
LANES = 128
NG = D // LANES
NKG = NG + 4
HP = 24
VP = 32
TQ = 512
CK = 128
NQB = S // TQ
NC = S // CK
NSTEP = H * NQB
UN = 8
BLAG = 1
DEPLAG = 3
TM1 = 256
NB1 = S // TM1
TM3 = 128
NB3 = S // TM3
STRADDLE = (6, 12, 19, 25)
QSCALE = float(DH) ** -0.5 * 1.4426950408889634

F32 = jnp.float32
BF16 = jnp.bfloat16
U32 = jnp.uint32


def _pack(x):
    return pltpu.bitcast(x, U32)


def _unpack(x):
    return pltpu.bitcast(x, BF16)


NT = (((1,), (1,)), ((), ()))
TN = (((0,), (0,)), ((), ()))


def _layernorm(x):
    mu = jnp.mean(x, axis=-1, keepdims=True)
    xc = x - mu
    var = jnp.mean(xc * xc, axis=-1, keepdims=True)
    return xc * lax.rsqrt(var + EPS)


def _gelu(x):
    c = 0.7978845608028654
    return 0.5 * x * (1.0 + jnp.tanh(c * (x + 0.044715 * (x * x * x))))


def _kernel(x_hbm, wqkv_hbm, wo_hbm, wg_hbm, wu_hbm, wd_hbm, c_hbm, wmod_hbm,
            out_hbm,
            x_v, wqkv_v, wo_v, wg_v, wu_v, wt_v, wd_v, c_v, wmod_v, out_v,
            mod_v, wqvt_v, h_all,
            h0, h1, x10, x11,
            k_s, qt_s, vt_s, s0, s1, m0, m1, q0, q1, at_s,
            in_sems, out_sems):
    def cp(src, dst, i):
        return pltpu.make_async_copy(src, dst, in_sems.at[i])

    XA = 2 * TM1

    xa_cp = cp(x_hbm.at[0:XA, :], x_v.at[0:XA, :], 12)
    xb_cp = cp(x_hbm.at[XA:S, :], x_v.at[XA:S, :], 13)
    c_cp = cp(c_hbm, c_v, 0)
    wmod_a = cp(wmod_hbm.at[:, 0:2 * D], wmod_v.at[:, 0:2 * D], 1)
    wk_cp = cp(wqkv_hbm.at[:, D:2 * D], wqkv_v.at[:, D:2 * D], 2)
    wq_cp = cp(wqkv_hbm.at[:, 0:D], wqkv_v.at[:, 0:D], 3)
    wv_cp = cp(wqkv_hbm.at[:, 2 * D:3 * D], wqkv_v.at[:, 2 * D:3 * D], 4)
    wmod_b = cp(wmod_hbm.at[:, 2 * D:6 * D], wmod_v.at[:, 2 * D:6 * D], 5)
    wo_cp = cp(wo_hbm, wo_v, 6)
    wg_cp = cp(wg_hbm, wg_v, 7)
    wu_cp = cp(wu_hbm, wu_v, 8)
    wd_cp = cp(wd_hbm, wd_v, 9)
    wtg_cp = cp(wg_hbm.at[FM:F, :], wt_v.at[0:FT, :], 10)
    wtu_cp = cp(wu_hbm.at[FM:F, :], wt_v.at[FT:2 * FT, :], 11)
    c_cp.start()
    wmod_a.start()
    xa_cp.start()
    wk_cp.start()

    c_cp.wait()
    cf = c_v[...].astype(F32)
    sc = (cf * jax.nn.sigmoid(cf)).astype(BF16)
    sc16 = jnp.broadcast_to(sc, (16, D))
    wmod_a.wait()
    xb_cp.start()
    mod_v[:, 0:2 * D] = jnp.dot(sc16, wmod_v[:, 0:2 * D], preferred_element_type=F32)

    TA = 128

    def ln1(r):
        rows = pl.ds(r * TA, TA)
        sa = mod_v[0:1, 0:D]
        ca = mod_v[0:1, D:2 * D]
        h_all[pl.ds(r * (TA // 2), TA // 2), :] = _pack(
            (_layernorm(x_v[rows, :].astype(F32)) * (1.0 + ca) + sa).astype(BF16))

    def kproj(r):
        prow = pl.ds(r * (TA // 2), TA // 2)
        kk = jnp.dot(_unpack(h_all[prow, :]), wqkv_v[:, D:2 * D], preferred_element_type=F32)
        kg = [kk[:, g * LANES:(g + 1) * LANES] for g in range(NG)]
        for g in range(NG):
            k_s[g, prow, :] = _pack(kg[g].astype(BF16))
        lane = lax.broadcasted_iota(jnp.int32, (TA, LANES), 1)
        for i, h in enumerate(STRADDLE):
            g, lo = divmod(h * DH, LANES)
            k_s[NG + i, prow, :] = _pack(jnp.where(lane >= lo, kg[g], kg[g + 1]).astype(BF16))

    xa_cp.wait()
    wk_cp.wait()
    wq_cp.start()
    wv_cp.start()
    for r in range(XA // TA):
        ln1(r)
        kproj(r)
    xb_cp.wait()
    NA = S // TA
    for r in range(XA // TA, NA):
        ln1(r)
        kproj(r)
        if r == NA - 5:
            wq_cp.wait()
            wv_cp.wait()
            wmod_b.start()
            wo_cp.start()
            wg_cp.start()
            wu_cp.start()
            wd_cp.start()
            wtg_cp.start()
            wtu_cp.start()
            wqvt_v[0:D // 2, :] = _pack(wqkv_v[:, 0:D].T)
            wqvt_v[D // 2:D, :] = _pack(wqkv_v[:, 2 * D:3 * D].T)

    def qvproj(r):
        rows = pl.ds(pl.multiple_of(r * TM1, TM1), TM1)
        prow = pl.ds(pl.multiple_of(r * (TM1 // 2), TM1 // 2), TM1 // 2)
        qv = lax.dot_general(_unpack(wqvt_v[...]), _unpack(h_all[prow, :]), NT, preferred_element_type=F32)
        q = qv[0:D, :] * QSCALE
        qt_s[:, rows] = q.astype(BF16)
        tail = jnp.where(lax.broadcasted_iota(jnp.int32, (VP - DH, TM1), 0) == 0, 1.0, 0.0).astype(F32)
        for h in range(H):
            v0 = D + h * DH
            vt_s[h, :, rows] = _pack(jnp.concatenate([qv[v0:v0 + DH, :], tail], axis=0).astype(BF16))

    def phase1b(j, carry):
        qvproj(2 * j)
        qvproj(2 * j + 1)
        return carry

    lax.fori_loop(0, NB1 // 2, phase1b, 0)

    wmod_b.wait()
    wo_cp.wait()
    wg_cp.wait()
    wu_cp.wait()
    wd_cp.wait()
    wtg_cp.wait()
    wtu_cp.wait()

    s_refs = (s0, s1)
    m_refs = (m0, m1)
    q_refs = (q0, q1)

    def k_group(h):
        g = (h * DH) // LANES
        straddle = (h * DH + DH - 1) // LANES != g
        return jnp.where(straddle, NG + g, g)

    def prep_q(i, q_ref):
        i = jnp.minimum(i, NSTEP - 1)
        h = i // NQB
        qb = i % NQB
        c0 = h * DH
        g = c0 // LANES
        g2 = (c0 + DH - 1) // LANES
        lo = c0 - g * LANES
        cols = pl.ds(pl.multiple_of(qb * TQ, TQ), TQ)
        qa = qt_s[pl.ds(pl.multiple_of(g * LANES, LANES), LANES), cols]
        qb_ = qt_s[pl.ds(pl.multiple_of(g2 * LANES, LANES), LANES), cols]
        row = lax.broadcasted_iota(jnp.int32, (LANES, TQ), 0)
        zero = jnp.zeros_like(qa)
        q_ref[...] = _pack(jnp.where((row >= lo) & (row < lo + DH), qa,
                                     jnp.where(row < lo + DH - LANES, qb_, zero)))

    def attn_block(i0, n, a_first, a_last, b_first, b_last, more):
        nslots = n * NC
        b_at = [[] for _ in range(nslots)]
        for u in range(b_first, b_last + 1):
            lag = 0 if u == 0 else BLAG
            for c in range(NC):
                b_at[min(u * NC + c + lag, nslots - 1)].append((u, c))
        mhist = []
        bstate = {}
        for u in range(n):
            a, b = (u + 1) % 2, u % 2
            run_a = a_first <= u <= a_last
            if run_a:
                if u + 1 <= a_last or more:
                    prep_q(i0 + u + 2, q_refs[b])
                g = k_group((i0 + u + 1) // NQB)
                macc = None
            for c in range(NC):
                t = u * NC + c
                if run_a:
                    kc = _unpack(k_s[g, c * (CK // 2):(c + 1) * (CK // 2), :])
                    s = jnp.dot(kc, _unpack(q_refs[a][...]), preferred_element_type=F32)
                    s_refs[a][c * CK:(c + 1) * CK, :] = s
                    mm = jnp.max(s.reshape(CK // 8, 8, TQ), axis=0)
                    macc = mm if macc is None else jnp.maximum(macc, mm)
                    mhist.append(macc)
                else:
                    mhist.append(None)
                for (ub, cb_) in b_at[t]:
                    bb = ub % 2
                    ib = i0 + ub
                    hb = ib // NQB
                    if cb_ == 0:
                        bstate[ub] = [jnp.broadcast_to(m_refs[bb][...], (8, TQ)), None]
                    mb, oacc = bstate[ub]
                    mbb = mb
                    if t >= DEPLAG and mhist[t - DEPLAG] is not None:
                        mbb = jnp.maximum(mb, jnp.minimum(mhist[t - DEPLAG], mb))
                    sc_ = s_refs[bb][cb_ * CK:(cb_ + 1) * CK, :].reshape(CK // 8, 8, TQ)
                    p = jnp.exp2(sc_ - mbb[None]).reshape(CK, TQ).astype(BF16)
                    o = jnp.dot(_unpack(vt_s[hb, :, cb_ * CK:(cb_ + 1) * CK]), p,
                                preferred_element_type=F32)
                    oacc = o if oacc is None else oacc + o
                    bstate[ub][1] = oacc
                    if cb_ == NC - 1:
                        cols = pl.ds(pl.multiple_of((ib % NQB) * TQ, TQ), TQ)
                        at_s[hb, :, cols] = oacc[0:HP, :] * (1.0 / oacc[DH:DH + 1, :])
            if run_a:
                m_refs[a][...] = jnp.max(macc, axis=0, keepdims=True)

    prep_q(0, q0)
    prep_q(1, q1)
    attn_block(-2, 2, 1, 1, 1, 0, False)

    def body(j, carry):
        attn_block(UN * j, UN, 0, UN - 1, 0, UN - 1, True)
        return carry

    lax.fori_loop(0, NSTEP // UN - 1, body, 0)
    attn_block(NSTEP - UN, UN, 0, UN - 2, 0, UN - 1, False)

    mod_v[:, 2 * D:6 * D] = jnp.dot(sc16, wmod_v[:, 2 * D:6 * D], preferred_element_type=F32)
    h_refs = (h0, h1)
    x1_refs = (x10, x11)

    def out_cp(blk):
        r0 = pl.multiple_of(blk * TM3, TM3)
        return pltpu.make_async_copy(out_v.at[pl.ds(r0, TM3), :], out_hbm.at[pl.ds(r0, TM3), :],
                                     out_sems.at[blk])

    def stage_x(blk, h_ref, x1_ref):
        blk = jnp.minimum(blk, NB3 - 1)
        rows = pl.ds(pl.multiple_of(blk * TM3, TM3), TM3)
        ga = mod_v[0:1, 2 * D:3 * D]
        sb = mod_v[0:1, 3 * D:4 * D]
        cb = mod_v[0:1, 4 * D:5 * D]
        a_t = jnp.concatenate([at_s[h, 0:DH, rows] for h in range(H)], axis=0).astype(BF16)
        y = lax.dot_general(a_t, wo_v[...], TN, preferred_element_type=F32)
        x1 = x_v[rows, :].astype(F32) + ga * y
        x1_ref[...] = x1
        h_ref[...] = _pack((_layernorm(x1) * (1.0 + cb) + sb).astype(BF16))

    def ffn_block(blk, h_ref, x1_ref, hn_ref, x1n_ref):
        rows = pl.ds(pl.multiple_of(blk * TM3, TM3), TM3)
        gb = mod_v[0:1, 5 * D:6 * D]
        h2 = _unpack(h_ref[...])

        def act_chunk(f0, f1):
            if f0 == FM:
                gu = lax.dot_general(h2, wt_v[...], NT, preferred_element_type=F32)
                return (_gelu(gu) * pltpu.roll(gu, FT, 1))[:, 0:FT].astype(BF16)
            gate = lax.dot_general(h2, wg_v[f0:f1, :], NT, preferred_element_type=F32)
            up = lax.dot_general(h2, wu_v[f0:f1, :], NT, preferred_element_type=F32)
            return (_gelu(gate) * up).astype(BF16)

        bounds = FCH
        y2 = None
        prev = None
        for n, (f0, f1) in enumerate(bounds):
            act = act_chunk(f0, f1)
            if n == XPOS:
                stage_x(blk + 1, hn_ref, x1n_ref)
            if prev is not None:
                d = jnp.dot(prev[0], wd_v[prev[1]:prev[2], :], preferred_element_type=F32)
                y2 = d if y2 is None else y2 + d
            prev = (act, f0, f1)
        y2 = y2 + jnp.dot(prev[0], wd_v[prev[1]:prev[2], :], preferred_element_type=F32)
        out_v[rows, :] = (x1_ref[...] + gb * y2).astype(BF16)
        out_cp(blk).start()

    stage_x(0, h0, x10)

    def phase3(j, carry):
        for u in range(2):
            ffn_block(2 * j + u, h_refs[u], x1_refs[u], h_refs[1 - u], x1_refs[1 - u])
        return carry

    lax.fori_loop(0, NB3 // 2, phase3, 0)

    for blk in range(NB3):
        out_cp(blk).wait()


@jax.jit
def pallas_adaLN_cond__mha_block__geglu_ffn__prompt_kernel(
    A_x: jax.Array,
    A_wqkv: jax.Array,
    A_wo: jax.Array,
    B_x: jax.Array,
    B_w_gate: jax.Array,
    B_w_up: jax.Array,
    B_w_down: jax.Array,
    c: jax.Array,
    w_mod: jax.Array,
):
    del B_x
    x = A_x.reshape(S, D)
    hbm = pl.BlockSpec(memory_space=pltpu.HBM)
    vm = pltpu.VMEM
    out = pl.pallas_call(
        _kernel,
        out_shape=jax.ShapeDtypeStruct((S, D), BF16),
        in_specs=[hbm] * 8,
        out_specs=hbm,
        scratch_shapes=[
            vm((S, D), BF16),
            vm((D, 3 * D), BF16),
            vm((D, D), BF16),
            vm((F, D), BF16),
            vm((F, D), BF16),
            vm((2 * FT, D), BF16),
            vm((F, D), BF16),
            vm((1, D), BF16),
            vm((D, 6 * D), BF16),
            vm((S, D), BF16),
            vm((16, 6 * D), F32),
            vm((D, D), U32),
            vm((S // 2, D), U32),
            vm((TM3 // 2, D), U32),
            vm((TM3 // 2, D), U32),
            vm((TM3, D), F32),
            vm((TM3, D), F32),
            vm((NKG, S // 2, LANES), U32),
            vm((D, S), BF16),
            vm((H, VP // 2, S), U32),
            vm((S, TQ), F32),
            vm((S, TQ), F32),
            vm((1, TQ), F32),
            vm((1, TQ), F32),
            vm((LANES // 2, TQ), U32),
            vm((LANES // 2, TQ), U32),
            vm((H, HP, S), F32),
            pltpu.SemaphoreType.DMA((14,)),
            pltpu.SemaphoreType.DMA((NB3,)),
        ],
        compiler_params=pltpu.CompilerParams(vmem_limit_bytes=100 * 1024 * 1024),
    )(x, A_wqkv, A_wo, B_w_gate.T, B_w_up.T, B_w_down, c, w_mod)
    return out.reshape(1, S, D)
```

```python
import jax
import jax.numpy as jnp
from jax import lax
import jax.experimental.pallas as pl
import jax.experimental.pallas.tpu as pltpu

S = 2048
D = 640
H = 32
DH = 20
F = 1728
FM = 1664
FT = F - FM
EPS = 1e-5
FCW = 256
XPOS = 2
FCH = [(FM, F)] + [(f, min(f + FCW, FM)) for f in range(0, FM, FCW)]
LANES = 128
NG = D // LANES
NKG = NG + 4
HP = 24
VP = 32
TQ = 512
CK = 128
NQB = S // TQ
NC = S // CK
NSTEP = H * NQB
UN = 8
BLAG = 1
DEPLAG = 3
XA = 640
TA = 128
NA = S // TA
TM1 = 256
NB1 = S // TM1
TM3 = 128
NB3 = S // TM3
STRADDLE = (6, 12, 19, 25)
QSCALE = float(DH) ** -0.5 * 1.4426950408889634

F32 = jnp.float32
BF16 = jnp.bfloat16
U32 = jnp.uint32


def _pack(x):
    return pltpu.bitcast(x, U32)


def _unpack(x):
    return pltpu.bitcast(x, BF16)


NT = (((1,), (1,)), ((), ()))
TN = (((0,), (0,)), ((), ()))


def _layernorm(x):
    mu = jnp.mean(x, axis=-1, keepdims=True)
    xc = x - mu
    var = jnp.mean(xc * xc, axis=-1, keepdims=True)
    return xc * lax.rsqrt(var + EPS)


def _gelu(x):
    c = 0.7978845608028654
    return 0.5 * x * (1.0 + jnp.tanh(c * (x + 0.044715 * (x * x * x))))


def _kernel(x_hbm, wqkv_hbm, wo_hbm, wg_hbm, wu_hbm, wd_hbm, c_hbm, wmod_hbm,
            out_hbm,
            x_v, wqkv_v, wo_v, wg_v, wu_v, wt_v, wd_v, c_v, wmod_v, out_v,
            mod_v, wqvt_v, h_all,
            h0, h1, x10, x11,
            k_s, qt_s, vt_s, s0, s1, m0, m1, q0, q1, at_s,
            in_sems, out_sems):
    def cp(src, dst, i):
        return pltpu.make_async_copy(src, dst, in_sems.at[i])

    xa_cp = cp(x_hbm.at[0:XA, :], x_v.at[0:XA, :], 12)
    xb_cp = cp(x_hbm.at[XA:S, :], x_v.at[XA:S, :], 13)
    c_cp = cp(c_hbm, c_v, 0)
    wmod_a = cp(wmod_hbm.at[:, 0:2 * D], wmod_v.at[:, 0:2 * D], 1)
    wk_cp = cp(wqkv_hbm.at[:, D:2 * D], wqkv_v.at[:, D:2 * D], 2)
    wq_cp = cp(wqkv_hbm.at[:, 0:D], wqkv_v.at[:, 0:D], 3)
    wv_cp = cp(wqkv_hbm.at[:, 2 * D:3 * D], wqkv_v.at[:, 2 * D:3 * D], 4)
    wmod_b = cp(wmod_hbm.at[:, 2 * D:6 * D], wmod_v.at[:, 2 * D:6 * D], 5)
    wo_cp = cp(wo_hbm, wo_v, 6)
    wg_cp = cp(wg_hbm, wg_v, 7)
    wu_cp = cp(wu_hbm, wu_v, 8)
    wd_cp = cp(wd_hbm, wd_v, 9)
    wtg_cp = cp(wg_hbm.at[FM:F, :], wt_v.at[0:FT, :], 10)
    wtu_cp = cp(wu_hbm.at[FM:F, :], wt_v.at[FT:2 * FT, :], 11)
    c_cp.start()
    wmod_a.start()
    xa_cp.start()
    wk_cp.start()

    c_cp.wait()
    cf = c_v[...].astype(F32)
    sc = (cf * jax.nn.sigmoid(cf)).astype(BF16)
    sc16 = jnp.broadcast_to(sc, (16, D))
    wmod_a.wait()
    xb_cp.start()
    mod_v[:, 0:2 * D] = jnp.dot(sc16, wmod_v[:, 0:2 * D], preferred_element_type=F32)

    def ln1(r):
        rows = pl.ds(r * TA, TA)
        sa = mod_v[0:1, 0:D]
        ca = mod_v[0:1, D:2 * D]
        h_all[pl.ds(r * (TA // 2), TA // 2), :] = _pack(
            (_layernorm(x_v[rows, :].astype(F32)) * (1.0 + ca) + sa).astype(BF16))

    def kproj(r):
        prow = pl.ds(r * (TA // 2), TA // 2)
        kk = jnp.dot(_unpack(h_all[prow, :]), wqkv_v[:, D:2 * D], preferred_element_type=F32)
        kg = [kk[:, g * LANES:(g + 1) * LANES] for g in range(NG)]
        for g in range(NG):
            k_s[g, prow, :] = _pack(kg[g].astype(BF16))
        lane = lax.broadcasted_iota(jnp.int32, (TA, LANES), 1)
        for i, h in enumerate(STRADDLE):
            g, lo = divmod(h * DH, LANES)
            k_s[NG + i, prow, :] = _pack(jnp.where(lane >= lo, kg[g], kg[g + 1]).astype(BF16))

    xa_cp.wait()
    wk_cp.wait()
    wq_cp.start()
    wv_cp.start()
    ln1(0)
    for r in range(NA):
        if r + 1 == XA // TA:
            xb_cp.wait()
        if r + 1 < NA and r + 1 != XA // TA:
            ln1(r + 1)
        if r == NA - 5:
            wq_cp.wait()
            wv_cp.wait()
            wmod_b.start()
            wo_cp.start()
            wg_cp.start()
            wu_cp.start()
            wd_cp.start()
            wtg_cp.start()
            wtu_cp.start()
            wqvt_v[0:D // 2, :] = _pack(wqkv_v[:, 0:D].T)
            wqvt_v[D // 2:D, :] = _pack(wqkv_v[:, 2 * D:3 * D].T)
        kproj(r)
        if r + 1 == XA // TA:
            ln1(r + 1)

    def qvproj(r):
        rows = pl.ds(pl.multiple_of(r * TM1, TM1), TM1)
        prow = pl.ds(pl.multiple_of(r * (TM1 // 2), TM1 // 2), TM1 // 2)
        qv = lax.dot_general(_unpack(wqvt_v[...]), _unpack(h_all[prow, :]), NT, preferred_element_type=F32)
        q = qv[0:D, :] * QSCALE
        qt_s[:, rows] = q.astype(BF16)
        tail = jnp.where(lax.broadcasted_iota(jnp.int32, (VP - DH, TM1), 0) == 0, 1.0, 0.0).astype(F32)
        for h in range(H):
            v0 = D + h * DH
            vt_s[h, :, rows] = _pack(jnp.concatenate([qv[v0:v0 + DH, :], tail], axis=0).astype(BF16))

    def phase1b(j, carry):
        qvproj(2 * j)
        qvproj(2 * j + 1)
        return carry

    lax.fori_loop(0, NB1 // 2, phase1b, 0)

    wmod_b.wait()
    wo_cp.wait()
    wg_cp.wait()
    wu_cp.wait()
    wd_cp.wait()
    wtg_cp.wait()
    wtu_cp.wait()

    def mod_rest():
        mod_v[:, 2 * D:6 * D] = jnp.dot(sc16, wmod_v[:, 2 * D:6 * D], preferred_element_type=F32)

    h_refs = (h0, h1)
    x1_refs = (x10, x11)

    def out_cp(blk):
        r0 = pl.multiple_of(blk * TM3, TM3)
        return pltpu.make_async_copy(out_v.at[pl.ds(r0, TM3), :], out_hbm.at[pl.ds(r0, TM3), :],
                                     out_sems.at[blk])

    def stage_x(blk, h_ref, x1_ref):
        blk = jnp.minimum(blk, NB3 - 1)
        rows = pl.ds(pl.multiple_of(blk * TM3, TM3), TM3)
        ga = mod_v[0:1, 2 * D:3 * D]
        sb = mod_v[0:1, 3 * D:4 * D]
        cb = mod_v[0:1, 4 * D:5 * D]
        a_t = jnp.concatenate([at_s[h, 0:DH, rows] for h in range(H)], axis=0).astype(BF16)
        y = lax.dot_general(a_t, wo_v[...], TN, preferred_element_type=F32)
        x1 = x_v[rows, :].astype(F32) + ga * y
        x1_ref[...] = x1
        h_ref[...] = _pack((_layernorm(x1) * (1.0 + cb) + sb).astype(BF16))

    s_refs = (s0, s1)
    m_refs = (m0, m1)
    q_refs = (q0, q1)

    def k_group(h):
        g = (h * DH) // LANES
        straddle = (h * DH + DH - 1) // LANES != g
        return jnp.where(straddle, NG + g, g)

    def prep_q(i, q_ref):
        i = jnp.minimum(i, NSTEP - 1)
        h = i // NQB
        qb = i % NQB
        c0 = h * DH
        g = c0 // LANES
        g2 = (c0 + DH - 1) // LANES
        lo = c0 - g * LANES
        cols = pl.ds(pl.multiple_of(qb * TQ, TQ), TQ)
        qa = qt_s[pl.ds(pl.multiple_of(g * LANES, LANES), LANES), cols]
        qb_ = qt_s[pl.ds(pl.multiple_of(g2 * LANES, LANES), LANES), cols]
        row = lax.broadcasted_iota(jnp.int32, (LANES, TQ), 0)
        zero = jnp.zeros_like(qa)
        q_ref[...] = _pack(jnp.where((row >= lo) & (row < lo + DH), qa,
                                     jnp.where(row < lo + DH - LANES, qb_, zero)))

    def attn_block(i0, n, a_first, a_last, b_first, b_last, more, extras=None):
        nslots = n * NC
        b_at = [[] for _ in range(nslots)]
        for u in range(b_first, b_last + 1):
            lag = 0 if u == 0 else BLAG
            for c in range(NC):
                b_at[min(u * NC + c + lag, nslots - 1)].append((u, c))
        mhist = []
        bstate = {}
        for u in range(n):
            a, b = (u + 1) % 2, u % 2
            run_a = a_first <= u <= a_last
            if run_a:
                if u + 1 <= a_last or more:
                    prep_q(i0 + u + 2, q_refs[b])
                g = k_group((i0 + u + 1) // NQB)
                macc = None
            for c in range(NC):
                t = u * NC + c
                if extras is not None and t in extras:
                    extras[t]()
                if run_a:
                    kc = _unpack(k_s[g, c * (CK // 2):(c + 1) * (CK // 2), :])
                    s = jnp.dot(kc, _unpack(q_refs[a][...]), preferred_element_type=F32)
                    s_refs[a][c * CK:(c + 1) * CK, :] = s
                    mm = jnp.max(s.reshape(CK // 8, 8, TQ), axis=0)
                    macc = mm if macc is None else jnp.maximum(macc, mm)
                    mhist.append(macc)
                else:
                    mhist.append(None)
                for (ub, cb_) in b_at[t]:
                    bb = ub % 2
                    ib = i0 + ub
                    hb = ib // NQB
                    if cb_ == 0:
                        bstate[ub] = [jnp.broadcast_to(m_refs[bb][...], (8, TQ)), None]
                    mb, oacc = bstate[ub]
                    mbb = mb
                    if t >= DEPLAG and mhist[t - DEPLAG] is not None:
                        mbb = jnp.maximum(mb, jnp.minimum(mhist[t - DEPLAG], mb))
                    sc_ = s_refs[bb][cb_ * CK:(cb_ + 1) * CK, :].reshape(CK // 8, 8, TQ)
                    p = jnp.exp2(sc_ - mbb[None]).reshape(CK, TQ).astype(BF16)
                    o = jnp.dot(_unpack(vt_s[hb, :, cb_ * CK:(cb_ + 1) * CK]), p,
                                preferred_element_type=F32)
                    oacc = o if oacc is None else oacc + o
                    bstate[ub][1] = oacc
                    if cb_ == NC - 1:
                        cols = pl.ds(pl.multiple_of((ib % NQB) * TQ, TQ), TQ)
                        at_s[hb, :, cols] = oacc[0:HP, :] * (1.0 / oacc[DH:DH + 1, :])
            if run_a:
                m_refs[a][...] = jnp.max(macc, axis=0, keepdims=True)

    prep_q(0, q0)
    prep_q(1, q1)
    attn_block(-2, 2, 1, 1, 1, 0, False)

    def body(j, carry):
        attn_block(UN * j, UN, 0, UN - 1, 0, UN - 1, True)
        return carry

    lax.fori_loop(0, NSTEP // UN - 1, body, 0)
    attn_block(NSTEP - UN, UN, 0, UN - 2, 0, UN - 1, False,
               extras={NC: mod_rest, (UN - 1) * NC: lambda: stage_x(0, h0, x10)})

    def ffn_block(blk, h_ref, x1_ref, hn_ref, x1n_ref):
        rows = pl.ds(pl.multiple_of(blk * TM3, TM3), TM3)
        gb = mod_v[0:1, 5 * D:6 * D]
        h2 = _unpack(h_ref[...])

        def act_chunk(f0, f1):
            if f0 == FM:
                gu = lax.dot_general(h2, wt_v[...], NT, preferred_element_type=F32)
                return (_gelu(gu) * pltpu.roll(gu, FT, 1))[:, 0:FT].astype(BF16)
            gate = lax.dot_general(h2, wg_v[f0:f1, :], NT, preferred_element_type=F32)
            up = lax.dot_general(h2, wu_v[f0:f1, :], NT, preferred_element_type=F32)
            return (_gelu(gate) * up).astype(BF16)

        y2 = None
        prev = None
        for n, (f0, f1) in enumerate(FCH):
            act = act_chunk(f0, f1)
            if n == XPOS:
                stage_x(blk + 1, hn_ref, x1n_ref)
            if prev is not None:
                d = jnp.dot(prev[0], wd_v[prev[1]:prev[2], :], preferred_element_type=F32)
                y2 = d if y2 is None else y2 + d
            prev = (act, f0, f1)
        y2 = y2 + jnp.dot(prev[0], wd_v[prev[1]:prev[2], :], preferred_element_type=F32)
        out_v[rows, :] = (x1_ref[...] + gb * y2).astype(BF16)
        out_cp(blk).start()

    def phase3(j, carry):
        for u in range(2):
            ffn_block(2 * j + u, h_refs[u], x1_refs[u], h_refs[1 - u], x1_refs[1 - u])
        return carry

    lax.fori_loop(0, NB3 // 2, phase3, 0)

    for blk in range(NB3):
        out_cp(blk).wait()


@jax.jit
def pallas_adaLN_cond__mha_block__geglu_ffn__prompt_kernel(
    A_x: jax.Array,
    A_wqkv: jax.Array,
    A_wo: jax.Array,
    B_x: jax.Array,
    B_w_gate: jax.Array,
    B_w_up: jax.Array,
    B_w_down: jax.Array,
    c: jax.Array,
    w_mod: jax.Array,
):
    del B_x
    x = A_x.reshape(S, D)
    hbm = pl.BlockSpec(memory_space=pltpu.HBM)
    vm = pltpu.VMEM
    out = pl.pallas_call(
        _kernel,
        out_shape=jax.ShapeDtypeStruct((S, D), BF16),
        in_specs=[hbm] * 8,
        out_specs=hbm,
        scratch_shapes=[
            vm((S, D), BF16),
            vm((D, 3 * D), BF16),
            vm((D, D), BF16),
            vm((F, D), BF16),
            vm((F, D), BF16),
            vm((2 * FT, D), BF16),
            vm((F, D), BF16),
            vm((1, D), BF16),
            vm((D, 6 * D), BF16),
            vm((S, D), BF16),
            vm((16, 6 * D), F32),
            vm((D, D), U32),
            vm((S // 2, D), U32),
            vm((TM3 // 2, D), U32),
            vm((TM3 // 2, D), U32),
            vm((TM3, D), F32),
            vm((TM3, D), F32),
            vm((NKG, S // 2, LANES), U32),
            vm((D, S), BF16),
            vm((H, VP // 2, S), U32),
            vm((S, TQ), F32),
            vm((S, TQ), F32),
            vm((1, TQ), F32),
            vm((1, TQ), F32),
            vm((LANES // 2, TQ), U32),
            vm((LANES // 2, TQ), U32),
            vm((H, HP, S), F32),
            pltpu.SemaphoreType.DMA((14,)),
            pltpu.SemaphoreType.DMA((NB3,)),
        ],
        compiler_params=pltpu.CompilerParams(vmem_limit_bytes=100 * 1024 * 1024),
    )(x, A_wqkv, A_wo, B_w_gate.T, B_w_up.T, B_w_down, c, w_mod)
    return out.reshape(1, S, D)
```
